```python
import jax
import jax.numpy as jnp

def _softmax(x, axis=-1):
    return jax.nn.softmax(x, axis=axis)
def _gelu(x):
    return jax.nn.gelu(x, approximate=True)
def _silu(x):
    return jax.nn.silu(x)
def _sigmoid(x):
    return jax.nn.sigmoid(x)
def _layernorm(x, axis=-1, eps=1e-5):
    m = jnp.mean(x, axis=axis, keepdims=True)
    v = jnp.var(x, axis=axis, keepdims=True)
    return (x - m) / jnp.sqrt(v + eps)
def _scatter_add(tgt, idx, src, axis=0):
    return tgt.at[idx].add(src)
def _segment_sum(src, seg, n):
    return jax.ops.segment_sum(src, seg, n)
class _Rng:
    def __init__(self, key):
        self._k = key
    def _next(self):
        self._k, sub = jax.random.split(self._k)
        return sub
    def normal(self, shape):
        return jax.random.normal(self._next(), shape, dtype=jnp.bfloat16)
    def randint(self, lo, hi, shape):
        return jax.random.randint(self._next(), shape, lo, hi, dtype=jnp.int32)
    def uniform(self, shape, lo=0.0, hi=1.0):
        return jax.random.uniform(self._next(), shape, jnp.bfloat16, lo, hi)
    def permutation(self, n):
        return jax.random.permutation(self._next(), n)


kernel_name = 'standalone__dcn_v2_cross__recsys'

def setup_inputs():
    _rng = _Rng(jax.random.key(int.from_bytes(__import__("os").urandom(4), "little")))
    _w = (lambda a: (lambda t: t.astype(jnp.bfloat16) if jnp.issubdtype(t.dtype, jnp.floating) else t)(jnp.asarray(a)))
    B, F, D, L = 16384, 26, 128, 6
    Din = min(F * D, 1024)
    return {
        "x0": _w((lambda *s: _rng.normal(s) * 0.05)(B, Din)),
        "ws": _w((lambda *s: _rng.normal(s) * 0.05)(L, Din, Din)),
        "bs": _w((lambda *s: _rng.normal(s) * 0.05)(L, Din)),
    }

def reference(x0, ws, bs):
    x = x0
    for l in range(ws.shape[0]):
        x = x0 * (x @ ws[l] + bs[l]) + x
    return x
```

```python
import jax
import jax.numpy as jnp
import jax.experimental.pallas as pl
import jax.experimental.pallas.tpu as pltpu


def _build(TM=384, H=256, XF32=False):
    def kernel(x_hbm, w_hbm, b_hbm, o_hbm, xh, oh, xbuf, obuf, wbuf, bbuf,
               hsem, xsem, osem, wsem):
        L = w_hbm.shape[0]
        n = (x_hbm.shape[0] - H) // TM

        def rows(i):
            return pl.ds(pl.multiple_of(H + i * TM, 128), TM)

        def xcopy(i, slot):
            return pltpu.make_async_copy(x_hbm.at[rows(i)], xbuf.at[slot], xsem.at[slot])

        def ocopy(i, slot):
            return pltpu.make_async_copy(obuf.at[slot], o_hbm.at[rows(i)], osem.at[slot])

        def wcopy(l):
            return pltpu.make_async_copy(w_hbm.at[l], wbuf.at[l], wsem.at[l])

        bcopy = pltpu.make_async_copy(b_hbm, bbuf, wsem.at[L])
        xhcopy = pltpu.make_async_copy(x_hbm.at[pl.ds(0, H)], xh, hsem.at[0])
        ohcopy = pltpu.make_async_copy(oh, o_hbm.at[pl.ds(0, H)], hsem.at[1])

        def layer(x0, x, w, b):
            y = jnp.dot(x.astype(jnp.bfloat16), w, preferred_element_type=jnp.float32)
            x = x0.astype(jnp.float32) * (y + b) + x.astype(jnp.float32)
            return x if XF32 else x.astype(jnp.bfloat16)

        xhcopy.start()
        wcopy(0).start()
        bcopy.start()
        for l in range(1, L):
            wcopy(l).start()
        xcopy(0, 0).start()
        xcopy(1, 1).start()
        xhcopy.wait()
        bcopy.wait()
        bias = bbuf[...].astype(jnp.float32)
        lid = jax.lax.broadcasted_iota(jnp.int32, bias.shape, 0)
        oh[...] = xh[...]

        def head(l, _):
            wcopy(l).wait()
            b = jnp.sum(jnp.where(lid == l, bias, 0.0), axis=0, keepdims=True)
            oh[...] = layer(xh[...], oh[...], wbuf[l], b).astype(oh.dtype)

        jax.lax.fori_loop(0, L, head, None)
        ohcopy.start()
        xcopy(0, 0).wait()

        def body(i, _):
            slot = i % 2
            x0 = xbuf[slot]
            x = x0
            for l in range(L):
                x = layer(x0, x, wbuf[l], bbuf[l:l + 1, :].astype(jnp.float32))
            obuf[slot] = x.astype(obuf.dtype)
            ocopy(i, slot).start()
            xcopy(jnp.minimum(i + 2, n - 1), slot).start()
            xcopy(jnp.minimum(i + 1, n - 1), 1 - slot).wait()

            @pl.when(i >= 1)
            def _():
                ocopy(i - 1, 1 - slot).wait()

        jax.lax.fori_loop(0, n, body, None)
        xcopy(n - 1, (n + 1) % 2).wait()
        ocopy(n - 1, (n - 1) % 2).wait()
        ohcopy.wait()

    def f(x0, ws, bs):
        B, D = x0.shape
        L = ws.shape[0]
        assert (B - H) % TM == 0 and (B - H) // TM >= 2
        any_spec = pl.BlockSpec(memory_space=pl.ANY)
        return pl.pallas_call(
            kernel,
            in_specs=[any_spec, any_spec, any_spec],
            out_specs=any_spec,
            out_shape=jax.ShapeDtypeStruct((B, D), x0.dtype),
            scratch_shapes=[
                pltpu.VMEM((H, D), x0.dtype),
                pltpu.VMEM((H, D), x0.dtype),
                pltpu.VMEM((2, TM, D), x0.dtype),
                pltpu.VMEM((2, TM, D), x0.dtype),
                pltpu.VMEM((L, D, D), ws.dtype),
                pltpu.VMEM((L, D), bs.dtype),
                pltpu.SemaphoreType.DMA((2,)),
                pltpu.SemaphoreType.DMA((2,)),
                pltpu.SemaphoreType.DMA((2,)),
                pltpu.SemaphoreType.DMA((L + 1,)),
            ],
            compiler_params=pltpu.CompilerParams(vmem_limit_bytes=64 * 2**20),
        )(x0, ws, bs)

    return f


@jax.jit
def pallas_standalone__dcn_v2_cross__recsys_kernel(
    x0: jax.Array,
    ws: jax.Array,
    bs: jax.Array,
):
    return _build()(x0, ws, bs)
```

```python
import jax, jax.numpy as jnp
import jax.experimental.pallas as pl
import jax.experimental.pallas.tpu as pltpu
F32=jnp.float32; BF=jnp.bfloat16

def quad(a):
    m,k=a.shape[0]//2,a.shape[1]//2
    return a[:m,:k],a[:m,k:],a[m:,:k],a[m:,k:]
def lhs_ops(a,d):
    if d==0: return [a.astype(BF)]
    a11,a12,a21,a22=quad(a)
    return [o for t in (a11+a22,a21+a22,a11,a22,a11+a12,a21-a11,a12-a22) for o in lhs_ops(t,d-1)]
def rhs_ops(b,d):
    if d==0: return [b.astype(BF)]
    b11,b12,b21,b22=quad(b)
    return [o for t in (b11+b22,b11,b12-b22,b21-b11,b22,b11+b12,b21+b22) for o in rhs_ops(t,d-1)]
def combine(ms,d):
    if d==0: return ms[0]
    s=len(ms)//7
    m1,m2,m3,m4,m5,m6,m7=[combine(ms[i*s:(i+1)*s],d-1) for i in range(7)]
    top=jnp.concatenate([m1+m4-m5+m7, m3+m5],axis=1)
    bot=jnp.concatenate([m2+m4, m1-m2+m3+m6],axis=1)
    return jnp.concatenate([top,bot],axis=0)

def _build(TM=640,H=384,DEPTH=2,CM=None):
    CM=CM or TM
    P=7**DEPTH
    def kernel(x_hbm,w_hbm,b_hbm,o_hbm,xh,oh,xbuf,obuf,wbuf,sbuf,bbuf,hsem,xsem,osem,wsem):
        L=w_hbm.shape[0]; n=(x_hbm.shape[0]-H)//TM
        rows=lambda i: pl.ds(pl.multiple_of(H+i*TM,128),TM)
        xcopy=lambda i,s: pltpu.make_async_copy(x_hbm.at[rows(i)],xbuf.at[s],xsem.at[s])
        ocopy=lambda i,s: pltpu.make_async_copy(obuf.at[s],o_hbm.at[rows(i)],osem.at[s])
        wcopy=lambda l: pltpu.make_async_copy(w_hbm.at[l],wbuf.at[l],wsem.at[l])
        bcopy=pltpu.make_async_copy(b_hbm,bbuf,wsem.at[L])
        xhcopy=pltpu.make_async_copy(x_hbm.at[pl.ds(0,H)],xh,hsem.at[0])
        ohcopy=pltpu.make_async_copy(oh,o_hbm.at[pl.ds(0,H)],hsem.at[1])
        xhcopy.start(); wcopy(0).start(); bcopy.start()
        for l in range(1,L): wcopy(l).start()
        xcopy(0,0).start(); xcopy(1,1).start()
        xhcopy.wait(); bcopy.wait()
        bias=bbuf[...].astype(F32)
        lid=jax.lax.broadcasted_iota(jnp.int32,bias.shape,0)
        oh[...]=xh[...]
        def head(l,_):
            wcopy(l).wait()
            b=jnp.sum(jnp.where(lid==l,bias,0.0),axis=0,keepdims=True)
            x=oh[...]
            y=jnp.dot(x,wbuf[l],preferred_element_type=F32)
            oh[...]=(xh[...].astype(F32)*(y+b)+x.astype(F32)).astype(oh.dtype)
            for p,o in enumerate(rhs_ops(wbuf[l].astype(F32),DEPTH)):
                sbuf[l,p]=o
        jax.lax.fori_loop(0,L,head,None)
        ohcopy.start(); xcopy(0,0).wait()
        def body(i,_):
            slot=i%2
            nc=TM//CM
            x0s=[xbuf[slot,c*CM:(c+1)*CM,:].astype(F32) for c in range(nc)]
            xs=list(x0s)
            for l in range(L):
                b=bbuf[l:l+1,:].astype(F32)
                for c in range(nc):
                    ms=[jnp.dot(a,sbuf[l,p],preferred_element_type=F32) for p,a in enumerate(lhs_ops(xs[c],DEPTH))]
                    xs[c]=x0s[c]*(combine(ms,DEPTH)+b)+xs[c]
            for c in range(nc):
                obuf[slot,c*CM:(c+1)*CM,:]=xs[c].astype(BF)
            ocopy(i,slot).start()
            xcopy(jnp.minimum(i+2,n-1),slot).start()
            xcopy(jnp.minimum(i+1,n-1),1-slot).wait()
            @pl.when(i>=1)
            def _(): ocopy(i-1,1-slot).wait()
        jax.lax.fori_loop(0,n,body,None)
        xcopy(n-1,(n+1)%2).wait(); ocopy(n-1,(n-1)%2).wait(); ohcopy.wait()
    def f(x0,ws,bs):
        B,D=x0.shape; L=ws.shape[0]; d=D>>DEPTH
        assert (B-H)%TM==0
        a=pl.BlockSpec(memory_space=pl.ANY)
        return pl.pallas_call(kernel,in_specs=[a,a,a],out_specs=a,out_shape=jax.ShapeDtypeStruct((B,D),x0.dtype),
          scratch_shapes=[pltpu.VMEM((H,D),BF),pltpu.VMEM((H,D),BF),pltpu.VMEM((2,TM,D),BF),pltpu.VMEM((2,TM,D),BF),
            pltpu.VMEM((L,D,D),BF),pltpu.VMEM((L,P,d,d),BF),pltpu.VMEM((L,D),BF),
            pltpu.SemaphoreType.DMA((2,)),pltpu.SemaphoreType.DMA((2,)),pltpu.SemaphoreType.DMA((2,)),pltpu.SemaphoreType.DMA((L+1,))],
          compiler_params=pltpu.CompilerParams(vmem_limit_bytes=110*2**20))(x0,ws,bs)
    return f


@jax.jit
def pallas_standalone__dcn_v2_cross__recsys_kernel(
    x0: jax.Array,
    ws: jax.Array,
    bs: jax.Array,
):
    return _build()(x0, ws, bs)
```

```python
import jax, jax.numpy as jnp
import jax.experimental.pallas as pl
import jax.experimental.pallas.tpu as pltpu
F32=jnp.float32; BF=jnp.bfloat16

def quad(a):
    m,k=a.shape[0]//2,a.shape[1]//2
    return a[:m,:k],a[:m,k:],a[m:,:k],a[m:,k:]
def lhs_ops(a,d):
    if d==0: return [a.astype(BF)]
    a11,a12,a21,a22=quad(a)
    return [o for t in (a11+a22,a21+a22,a11,a22,a11+a12,a21-a11,a12-a22) for o in lhs_ops(t,d-1)]
def rhs_ops(b,d):
    if d==0: return [b.astype(BF)]
    b11,b12,b21,b22=quad(b)
    return [o for t in (b11+b22,b11,b12-b22,b21-b11,b22,b11+b12,b21+b22) for o in rhs_ops(t,d-1)]
def combine(ms,d):
    if d==0: return ms[0]
    s=len(ms)//7
    m1,m2,m3,m4,m5,m6,m7=[combine(ms[i*s:(i+1)*s],d-1) for i in range(7)]
    top=jnp.concatenate([m1+m4-m5+m7, m3+m5],axis=1)
    bot=jnp.concatenate([m2+m4, m1-m2+m3+m6],axis=1)
    return jnp.concatenate([top,bot],axis=0)

def _build(TM=512,CM=512,G=6,DEPTH=2):
    P=7**DEPTH; nc=TM//CM
    def kernel(x_hbm,w_hbm,b_hbm,o_hbm,xbuf,obuf,xs,wbuf,sbuf,bbuf,xsem,osem,wsem):
        L=w_hbm.shape[0]; n=x_hbm.shape[0]//TM
        rows=lambda i: pl.ds(pl.multiple_of(i*TM,128),TM)
        xcopy=lambda i,s: pltpu.make_async_copy(x_hbm.at[rows(i)],xbuf.at[s],xsem.at[s])
        ocopy=lambda i,s: pltpu.make_async_copy(obuf.at[s],o_hbm.at[rows(i)],osem.at[s])
        wcopy=lambda l: pltpu.make_async_copy(w_hbm.at[l],wbuf.at[l],wsem.at[l])
        bcopy=pltpu.make_async_copy(b_hbm,bbuf,wsem.at[L])
        for l in range(L): wcopy(l).start()
        bcopy.start(); xcopy(0,0).start(); xcopy(1,1).start()
        def pre(l,_):
            wcopy(l).wait()
            for p,o in enumerate(rhs_ops(wbuf[l].astype(F32),DEPTH)): sbuf[l,p]=o
        jax.lax.fori_loop(0,L,pre,None)
        bcopy.wait(); xcopy(0,0).wait()
        bias=bbuf[...].astype(F32)
        lid=jax.lax.broadcasted_iota(jnp.int32,bias.shape,0)
        def body(i,_):
            slot=i%2
            if G<L: xs[...]=xbuf[slot].astype(F32)
            def group(g,_):
                x0s=[xbuf[slot,c*CM:(c+1)*CM,:].astype(F32) for c in range(nc)]
                v=[xs[c*CM:(c+1)*CM,:] for c in range(nc)] if G<L else list(x0s)
                for j in range(G):
                    l=g*G+j
                    b=jnp.sum(jnp.where(lid==l,bias,0.0),axis=0,keepdims=True)
                    for c in range(nc):
                        ms=[jnp.dot(a,sbuf[l,p],preferred_element_type=F32) for p,a in enumerate(lhs_ops(v[c],DEPTH))]
                        v[c]=x0s[c]*(combine(ms,DEPTH)+b)+v[c]
                for c in range(nc): xs[c*CM:(c+1)*CM,:]=v[c]
            if G<L: jax.lax.fori_loop(0,L//G,group,None)
            else: group(0,None)
            obuf[slot]=xs[...].astype(BF)
            ocopy(i,slot).start()
            xcopy(jnp.minimum(i+2,n-1),slot).start()
            xcopy(jnp.minimum(i+1,n-1),1-slot).wait()
            @pl.when(i>=1)
            def _(): ocopy(i-1,1-slot).wait()
        jax.lax.fori_loop(0,n,body,None)
        xcopy(n-1,(n+1)%2).wait(); ocopy(n-1,(n-1)%2).wait()
    def f(x0,ws,bs):
        B,D=x0.shape; L=ws.shape[0]; d=D>>DEPTH
        assert B%TM==0 and L%G==0
        a=pl.BlockSpec(memory_space=pl.ANY)
        return pl.pallas_call(kernel,in_specs=[a,a,a],out_specs=a,out_shape=jax.ShapeDtypeStruct((B,D),x0.dtype),
          scratch_shapes=[pltpu.VMEM((2,TM,D),BF),pltpu.VMEM((2,TM,D),BF),pltpu.VMEM((TM,D),F32),
            pltpu.VMEM((L,D,D),BF),pltpu.VMEM((L,P,d,d),BF),pltpu.VMEM((L,D),BF),
            pltpu.SemaphoreType.DMA((2,)),pltpu.SemaphoreType.DMA((2,)),pltpu.SemaphoreType.DMA((L+1,))],
          compiler_params=pltpu.CompilerParams(vmem_limit_bytes=110*2**20))(x0,ws,bs)
    return f


@jax.jit
def pallas_standalone__dcn_v2_cross__recsys_kernel(
    x0: jax.Array,
    ws: jax.Array,
    bs: jax.Array,
):
    return _build()(x0, ws, bs)
```
